```python
import jax
import jax.numpy as jnp

def _softmax(x, axis=-1):
    return jax.nn.softmax(x, axis=axis)
def _gelu(x):
    return jax.nn.gelu(x, approximate=True)
def _silu(x):
    return jax.nn.silu(x)
def _sigmoid(x):
    return jax.nn.sigmoid(x)
def _layernorm(x, axis=-1, eps=1e-5):
    m = jnp.mean(x, axis=axis, keepdims=True)
    v = jnp.var(x, axis=axis, keepdims=True)
    return (x - m) / jnp.sqrt(v + eps)
def _scatter_add(tgt, idx, src, axis=0):
    return tgt.at[idx].add(src)
def _segment_sum(src, seg, n):
    return jax.ops.segment_sum(src, seg, n)
class _Rng:
    def __init__(self, key):
        self._k = key
    def _next(self):
        self._k, sub = jax.random.split(self._k)
        return sub
    def normal(self, shape):
        return jax.random.normal(self._next(), shape, dtype=jnp.bfloat16)
    def randint(self, lo, hi, shape):
        return jax.random.randint(self._next(), shape, lo, hi, dtype=jnp.int32)
    def uniform(self, shape, lo=0.0, hi=1.0):
        return jax.random.uniform(self._next(), shape, jnp.bfloat16, lo, hi)
    def permutation(self, n):
        return jax.random.permutation(self._next(), n)


kernel_name = 'sequential_preLN__mha_block_cached__moe_arch_mod__decode'

def setup_inputs():
    _rng = _Rng(jax.random.key(int.from_bytes(__import__("os").urandom(4), "little")))
    _w = (lambda a: (lambda t: t.astype(jnp.bfloat16) if jnp.issubdtype(t.dtype, jnp.floating) else t)(jnp.asarray(a)))
    def _A_setup():
        B, Sq, D = 4, 1, 640
        H, Sk, Dh = 32, 8192, 192
        return {
            "x": _w((lambda *s: _rng.normal(s) * 0.05)(B, Sq, D)),
            "k_cache": _w((lambda *s: _rng.normal(s) * 0.05)(B, H, Sk, Dh)),
            "v_cache": _w((lambda *s: _rng.normal(s) * 0.05)(B, H, Sk, Dh)),
            "wq": _w((lambda *s: _rng.normal(s) * 0.05)(D, H * Dh) * (D ** -0.5)),
            "wo": _w((lambda *s: _rng.normal(s) * 0.05)(H * Dh, D) * ((H * Dh) ** -0.5)),
        }
    _A_in = _A_setup()

    def _B_setup():
        B, S, D, F, C = 4, 1, 640, 1536, 1
        return {
            "x": _w((lambda *s: _rng.normal(s) * 0.05)(B, S, D)),
            "w_r": _w((lambda *s: _rng.normal(s) * 0.05)(D)),
            "w_gate": _w((lambda *s: _rng.normal(s) * 0.05)(D, F)),
            "w_up": _w((lambda *s: _rng.normal(s) * 0.05)(D, F)),
            "w_down": _w((lambda *s: _rng.normal(s) * 0.05)(F, D)),
        }
    _B_in = _B_setup()

    return {
        "A_x": _A_in["x"],
        "A_k_cache": _A_in["k_cache"],
        "A_v_cache": _A_in["v_cache"],
        "A_wq": _A_in["wq"],
        "A_wo": _A_in["wo"],
        "B_x": _B_in["x"],
        "B_w_r": _B_in["w_r"],
        "B_w_gate": _B_in["w_gate"],
        "B_w_up": _B_in["w_up"],
        "B_w_down": _B_in["w_down"],
    }

def reference(A_x, A_k_cache, A_v_cache, A_wq, A_wo, B_x, B_w_r, B_w_gate, B_w_up, B_w_down):
    def _A_ref(x, k_cache, v_cache, wq, wo):
        B, Sq, D = x.shape
        H, Dh = 32, 192
        q = (lambda x, *d: x.transpose(*d))((x @ wq).reshape(B, Sq, H, Dh), 0, 2, 1, 3)
        scores = jnp.einsum("bhqd,bhkd->bhqk", q, k_cache) * (Dh ** -0.5)
        p = _softmax(scores, axis=-1)
        o = jnp.einsum("bhqk,bhkd->bhqd", p, v_cache)
        return (lambda x, *d: x.transpose(*d))(o, 0, 2, 1, 3).reshape(B, Sq, H * Dh) @ wo

    def _B_ref(x, w_r, w_gate, w_up, w_down):
        B, S, D = x.shape
        C = 1
        r = x @ w_r
        idx = jnp.argsort(-r, axis=-1)[:, :C]
        idx_e = jnp.repeat(idx.reshape(B, C, 1), D, axis=2)
        x_sel = jnp.take_along_axis(x, idx_e, axis=1)
        g = _silu(x_sel @ w_gate)
        u = x_sel @ w_up
        y = (g * u) @ w_down
        r_sel = _sigmoid(jnp.take_along_axis(r, idx, axis=1))
        y = y * r_sel.reshape(B, C, 1)
        b_off = (jnp.arange(B) * S).reshape(B, 1)
        flat_idx = (idx + b_off).reshape(B * C)
        zero = (x * 0.0).reshape(B * S, D)
        upd = _scatter_add(zero, flat_idx, y.reshape(B * C, D), axis=0)
        return x + upd.reshape(B, S, D)

    x = A_x
    h = x + _A_ref(_layernorm(x, axis=-1), A_k_cache, A_v_cache, A_wq, A_wo)
    h2 = h + _B_ref(_layernorm(h, axis=-1), B_w_r, B_w_gate, B_w_up, B_w_down)
    return h2
```

```python
import functools

import jax
import jax.numpy as jnp
import jax.experimental.pallas as pl
import jax.experimental.pallas.tpu as pltpu

_EPS = 1e-5
_ROWS = 8
_NB = 2
_CW = 256


def _layernorm(x):
    m = jnp.mean(x, axis=-1, keepdims=True)
    d = x - m
    v = jnp.mean(d * d, axis=-1, keepdims=True)
    return d / jnp.sqrt(v + _EPS)


def _dot(a, b):
    return jnp.dot(a, b, preferred_element_type=jnp.float32)


def _dot_nt(a, b):
    return jax.lax.dot_general(
        a, b, (((1,), (1,)), ((), ())), preferred_element_type=jnp.float32
    )


def _wait_all(buf, sem):
    pltpu.make_async_copy(buf, buf, sem).wait()


def _body(
    x_hbm, kt_hbm, vt_hbm, wq_hbm, wo_hbm, wr_hbm, wg_hbm, wu_hbm, wd_hbm,
    out_ref,
    kbuf, vbuf, wqbuf, wobuf, wgbuf, wubuf, wdbuf, xbuf, wrbuf, q_scr, o_scr,
    ksem, vsem, wqsem, wosem, msem,
    *, B, H, Dh, Sk, D, F,
):
    n_pairs = H // 2
    per_pair = 2 * B
    n_steps = n_pairs * per_pair
    scale = Dh ** -0.5

    def issue_kv(t):
        j = t % per_pair
        n = (j % B) * H + 2 * (t // per_pair) + j // B
        slot = t % _NB

        def piece(c, carry):
            cols = pl.ds(pl.multiple_of(c * _CW, _CW), _CW)
            pltpu.make_async_copy(
                kt_hbm.at[n, :, cols], kbuf.at[slot, :, cols], ksem.at[slot]
            ).start(priority=0)
            pltpu.make_async_copy(
                vt_hbm.at[n, :, cols], vbuf.at[slot, :, cols], vsem.at[slot]
            ).start(priority=1)
            return carry

        jax.lax.fori_loop(0, Sk // _CW, piece, None)

    def issue_wq(p):
        cols = pl.ds(pl.multiple_of(p * 2 * Dh, 2 * Dh), 2 * Dh)
        for i, r in enumerate(range(0, D, 128)):
            pltpu.make_async_copy(
                wq_hbm.at[pl.ds(r, 128), cols], wqbuf.at[pl.ds(r, 128), :], wqsem.at[0]
            ).start(priority=i % 2)

    def issue_wo(p):
        for i, r in enumerate(range(0, 2 * Dh, 64)):
            pltpu.make_async_copy(
                wo_hbm.at[pl.ds(pl.multiple_of(p * 2 * Dh + r, 64), 64), :],
                wobuf.at[pl.ds(r, 64), :],
                wosem.at[0],
            ).start(priority=(i + 1) % 2)

    def issue_gate_up():
        def piece(c, carry):
            rows = pl.ds(pl.multiple_of(c * 32, 32), 32)
            pltpu.make_async_copy(wg_hbm.at[rows, :], wgbuf.at[rows, :], msem.at[2]).start(priority=0)
            pltpu.make_async_copy(wu_hbm.at[rows, :], wubuf.at[rows, :], msem.at[3]).start(priority=1)
            return carry

        jax.lax.fori_loop(0, D // 32, piece, None)

    def issue_down():
        def piece(c, carry):
            for pr in range(2):
                rows = pl.ds(pl.multiple_of(c * 128 + pr * 64, 64), 64)
                pltpu.make_async_copy(wd_hbm.at[rows, :], wdbuf.at[rows, :], msem.at[4]).start(priority=pr)
            return carry

        jax.lax.fori_loop(0, F // 128, piece, None)

    x_cp = pltpu.make_async_copy(x_hbm, xbuf, msem.at[0])
    wr_cp = pltpu.make_async_copy(wr_hbm, wrbuf, msem.at[1])
    x_cp.start()
    issue_wq(0)
    wr_cp.start(priority=1)
    issue_kv(0)

    x_cp.wait()
    x = jnp.concatenate(
        [xbuf[...].astype(jnp.float32), jnp.zeros((_ROWS - B, D), jnp.float32)], axis=0
    )
    xn = _layernorm(x).astype(jnp.bfloat16)
    row = jax.lax.broadcasted_iota(jnp.int32, (_ROWS, Dh), 0)
    o_scr[...] = jnp.zeros_like(o_scr)

    for t in range(1, _NB):
        issue_kv(t)

    def step(t, attn):
        p = t // per_pair
        j = t % per_pair
        hh = j // B
        b = j % B
        slot = t % _NB

        @pl.when(j == 0)
        def _():
            issue_wo(p)
            _wait_all(wqbuf, wqsem.at[0])
            q = _dot(xn, wqbuf[...])
            q_scr[0] = q[:, :Dh]
            q_scr[1] = q[:, Dh:]

            @pl.when(p + 1 < n_pairs)
            def _():
                issue_wq(p + 1)

        _wait_all(kbuf.at[slot], ksem.at[slot])
        s = _dot(q_scr[hh].astype(jnp.bfloat16), kbuf[slot]) * scale
        e = jnp.exp(s - jnp.max(s, axis=-1, keepdims=True))
        l = jnp.sum(e, axis=-1, keepdims=True)
        _wait_all(vbuf.at[slot], vsem.at[slot])
        o = _dot_nt(e.astype(jnp.bfloat16), vbuf[slot]) / l
        o_scr[hh] = jnp.where(row == b, o, o_scr[hh])

        @pl.when(t + _NB < n_steps)
        def _():
            issue_kv(t + _NB)

        @pl.when(t + _NB == n_steps)
        def _():
            issue_gate_up()
            issue_down()

        def project():
            _wait_all(wobuf, wosem.at[0])
            return (
                attn
                + _dot(o_scr[0].astype(jnp.bfloat16), wobuf[:Dh, :])
                + _dot(o_scr[1].astype(jnp.bfloat16), wobuf[Dh:, :])
            )

        return jax.lax.cond(j == per_pair - 1, project, lambda: attn)

    attn = jax.lax.fori_loop(0, n_steps, step, jnp.zeros((_ROWS, D), jnp.float32))

    h = x + attn
    hn = _layernorm(h)
    hb = hn.astype(jnp.bfloat16)
    wr_cp.wait()
    r = jnp.sum(hn * wrbuf[...].astype(jnp.float32), axis=-1, keepdims=True)
    _wait_all(wgbuf, msem.at[2])
    _wait_all(wubuf, msem.at[3])
    g = _dot(hb, wgbuf[...])
    u = _dot(hb, wubuf[...])
    a = (g * jax.nn.sigmoid(g) * u).astype(jnp.bfloat16)
    _wait_all(wdbuf, msem.at[4])
    y = _dot(a, wdbuf[...]) * jax.nn.sigmoid(r)
    out = h + (hn + (hn * 0.0 + y))
    out_ref[...] = out[:B].astype(out_ref.dtype)


@jax.jit
def pallas_sequential_preLN__mha_block_cached__moe_arch_mod__decode_kernel(
    A_x: jax.Array,
    A_k_cache: jax.Array,
    A_v_cache: jax.Array,
    A_wq: jax.Array,
    A_wo: jax.Array,
    B_x: jax.Array,
    B_w_r: jax.Array,
    B_w_gate: jax.Array,
    B_w_up: jax.Array,
    B_w_down: jax.Array,
):
    del B_x
    B, Sq, D = A_x.shape
    _, H, Sk, Dh = A_k_cache.shape
    F = B_w_gate.shape[1]
    assert Sq == 1 and B <= _ROWS and H % 2 == 0 and Sk % _CW == 0
    dt = A_k_cache.dtype

    kt = jnp.swapaxes(A_k_cache, 2, 3).reshape(B * H, Dh, Sk)
    vt = jnp.swapaxes(A_v_cache, 2, 3).reshape(B * H, Dh, Sk)

    out = pl.pallas_call(
        functools.partial(_body, B=B, H=H, Dh=Dh, Sk=Sk, D=D, F=F),
        in_specs=[pl.BlockSpec(memory_space=pl.ANY)] * 9,
        out_specs=pl.BlockSpec(memory_space=pltpu.VMEM),
        out_shape=jax.ShapeDtypeStruct((B, D), A_x.dtype),
        scratch_shapes=[
            pltpu.VMEM((_NB, Dh, Sk), dt),
            pltpu.VMEM((_NB, Dh, Sk), dt),
            pltpu.VMEM((D, 2 * Dh), dt),
            pltpu.VMEM((2 * Dh, D), dt),
            pltpu.VMEM((D, F), dt),
            pltpu.VMEM((D, F), dt),
            pltpu.VMEM((F, D), dt),
            pltpu.VMEM((B, D), dt),
            pltpu.VMEM((1, D), dt),
            pltpu.VMEM((2, _ROWS, Dh), jnp.float32),
            pltpu.VMEM((2, _ROWS, Dh), jnp.float32),
            pltpu.SemaphoreType.DMA((_NB,)),
            pltpu.SemaphoreType.DMA((_NB,)),
            pltpu.SemaphoreType.DMA((1,)),
            pltpu.SemaphoreType.DMA((1,)),
            pltpu.SemaphoreType.DMA((5,)),
        ],
        compiler_params=pltpu.CompilerParams(vmem_limit_bytes=64 * 1024 * 1024),
    )(
        A_x.reshape(B, D), kt, vt, A_wq, A_wo, B_w_r.reshape(1, D),
        B_w_gate, B_w_up, B_w_down,
    )
    return out.reshape(B, Sq, D)
```

```python
import functools

import jax
import jax.numpy as jnp
import jax.experimental.pallas as pl
import jax.experimental.pallas.tpu as pltpu

_EPS = 1e-5
_NB = 3
_GW = 2048
_CW = 256
_CR = 96


def _layernorm(x):
    m = jnp.mean(x, axis=-1, keepdims=True)
    d = x - m
    v = jnp.mean(d * d, axis=-1, keepdims=True)
    return d / jnp.sqrt(v + _EPS)


def _dot(a, b):
    return jnp.dot(a, b, preferred_element_type=jnp.float32)


def _dot_nt(a, b):
    return jax.lax.dot_general(
        a, b, (((1,), (1,)), ((), ())), preferred_element_type=jnp.float32
    )


def _wait_all(buf, sem):
    pltpu.make_async_copy(buf, buf, sem).wait()


def _body(
    x_hbm, kt_hbm, vt_hbm, wq_hbm, wo_hbm, wr_hbm, wg_hbm, wu_hbm, wd_hbm,
    out_ref,
    kbuf, vbuf, wqbuf, wobuf, wgbuf, wubuf, wdbuf, xbuf, wrbuf,
    q_scr, o_scr, acc_scr, m_scr, l_scr, attn_scr,
    ksem, vsem, wqsem, wosem, msem,
    *, B, H, Dh, Sk, D, F,
):
    P = 2 * Dh
    n_pairs = H // 2
    G = Sk // _GW
    per_pair = B * G
    n_steps = n_pairs * per_pair
    scale = Dh ** -0.5

    def issue_kv(t):
        j = t % per_pair
        n = (j // G) * n_pairs + t // per_pair
        c0 = (j % G) * _GW
        slot = t % _NB

        def strip(c, carry):
            dst = pl.ds(pl.multiple_of(c * _CW, _CW), _CW)
            src = pl.ds(pl.multiple_of(c0 + c * _CW, _CW), _CW)
            for r in range(0, P, _CR):
                rows = pl.ds(r, _CR)
                pltpu.make_async_copy(
                    kt_hbm.at[n, rows, src], kbuf.at[slot, rows, dst], ksem.at[slot]
                ).start(priority=0)
                pltpu.make_async_copy(
                    vt_hbm.at[n, rows, src], vbuf.at[slot, rows, dst], vsem.at[slot]
                ).start(priority=1)
            return carry

        jax.lax.fori_loop(0, _GW // _CW, strip, None)

    def issue_wq(p):
        cols = pl.ds(pl.multiple_of(p * P, P), P)
        for i, r in enumerate(range(0, D, 64)):
            pltpu.make_async_copy(
                wq_hbm.at[pl.ds(r, 64), cols], wqbuf.at[pl.ds(r, 64), :], wqsem.at[0]
            ).start(priority=i % 2)

    def issue_wo(p):
        for i, r in enumerate(range(0, P, 32)):
            pltpu.make_async_copy(
                wo_hbm.at[pl.ds(pl.multiple_of(p * P + r, 32), 32), :],
                wobuf.at[pl.ds(r, 32), :],
                wosem.at[0],
            ).start(priority=i % 2)

    def issue_gate_up():
        def piece(c, carry):
            rows = pl.ds(pl.multiple_of(c * 32, 32), 32)
            pltpu.make_async_copy(wg_hbm.at[rows, :], wgbuf.at[rows, :], msem.at[2]).start(priority=0)
            pltpu.make_async_copy(wu_hbm.at[rows, :], wubuf.at[rows, :], msem.at[3]).start(priority=1)
            return carry

        jax.lax.fori_loop(0, D // 32, piece, None)

    def issue_down():
        def piece(c, carry):
            for pr in range(2):
                rows = pl.ds(pl.multiple_of(c * 128 + pr * 64, 64), 64)
                pltpu.make_async_copy(wd_hbm.at[rows, :], wdbuf.at[rows, :], msem.at[4]).start(priority=pr)
            return carry

        jax.lax.fori_loop(0, F // 128, piece, None)

    x_cp = pltpu.make_async_copy(x_hbm, xbuf, msem.at[0])
    wr_cp = pltpu.make_async_copy(wr_hbm, wrbuf, msem.at[1])
    x_cp.start()
    wr_cp.start(priority=1)
    issue_wq(0)
    issue_kv(0)

    x_cp.wait()
    x4 = xbuf[...].astype(jnp.float32)
    x = jnp.concatenate([x4, x4], axis=0)
    xn = _layernorm(x).astype(jnp.bfloat16)
    row = jax.lax.broadcasted_iota(jnp.int32, (2 * B, P), 0)
    col = jax.lax.broadcasted_iota(jnp.int32, (2 * B, P), 1)
    diag = (row < B) == (col < Dh)
    attn_scr[...] = jnp.zeros_like(attn_scr)
    o_scr[...] = jnp.zeros_like(o_scr)

    for t in range(1, _NB):
        issue_kv(t)

    def step(t, carry):
        p = t // per_pair
        j = t % per_pair
        b = j // G
        g = j % G
        slot = t % _NB

        @pl.when(j == 0)
        def _():
            issue_wo(p)
            _wait_all(wqbuf, wqsem.at[0])
            q_scr[...] = jnp.where(diag, _dot(xn, wqbuf[...]), 0.0)

            @pl.when(p + 1 < n_pairs)
            def _():
                issue_wq(p + 1)

        @pl.when(g == 0)
        def _():
            m_scr[...] = jnp.full_like(m_scr, -jnp.inf)
            l_scr[...] = jnp.zeros_like(l_scr)
            acc_scr[...] = jnp.zeros_like(acc_scr)

        _wait_all(kbuf.at[slot], ksem.at[slot])
        _wait_all(vbuf.at[slot], vsem.at[slot])
        s = _dot(q_scr[...].astype(jnp.bfloat16), kbuf[slot]) * scale
        m_old = m_scr[...]
        m_new = jnp.maximum(m_old, jnp.max(s, axis=-1, keepdims=True))
        m_sub = jnp.where(m_new == -jnp.inf, 0.0, m_new)
        e = jnp.exp(s - m_sub)
        alpha = jnp.exp(m_old - m_sub)
        m_scr[...] = m_new
        l_scr[...] = alpha * l_scr[...] + jnp.sum(e, axis=-1, keepdims=True)
        acc_scr[...] = alpha * acc_scr[...] + _dot_nt(e.astype(jnp.bfloat16), vbuf[slot])

        @pl.when(t + _NB < n_steps)
        def _():
            issue_kv(t + _NB)

        @pl.when(t + _NB == n_steps)
        def _():
            issue_gate_up()

        @pl.when(t + 1 == n_steps)
        def _():
            issue_down()

        @pl.when(g == G - 1)
        def _():
            o = jnp.where(diag, acc_scr[...] / l_scr[...], 0.0)
            o_scr[...] = jnp.where(row % B == b, o, o_scr[...])

        @pl.when(j == per_pair - 1)
        def _():
            _wait_all(wobuf, wosem.at[0])
            attn_scr[...] += _dot(o_scr[...].astype(jnp.bfloat16), wobuf[...])

        return carry

    jax.lax.fori_loop(0, n_steps, step, None)

    attn = attn_scr[...]
    h = x + attn + pltpu.roll(attn, B, 0)
    hn = _layernorm(h)
    hb = hn.astype(jnp.bfloat16)
    wr_cp.wait()
    r = jnp.sum(hn * wrbuf[...].astype(jnp.float32).reshape(1, D), axis=-1, keepdims=True)
    _wait_all(wgbuf, msem.at[2])
    _wait_all(wubuf, msem.at[3])
    gate = _dot(hb, wgbuf[...])
    up = _dot(hb, wubuf[...])
    act = (gate * jax.nn.sigmoid(gate) * up).astype(jnp.bfloat16)
    _wait_all(wdbuf, msem.at[4])
    y = _dot(act, wdbuf[...]) * jax.nn.sigmoid(r)
    out = h + (hn + (hn * 0.0 + y))
    out_ref[...] = out[:B].astype(out_ref.dtype)


@jax.jit
def pallas_sequential_preLN__mha_block_cached__moe_arch_mod__decode_kernel(
    A_x: jax.Array,
    A_k_cache: jax.Array,
    A_v_cache: jax.Array,
    A_wq: jax.Array,
    A_wo: jax.Array,
    B_x: jax.Array,
    B_w_r: jax.Array,
    B_w_gate: jax.Array,
    B_w_up: jax.Array,
    B_w_down: jax.Array,
):
    del B_x
    B, Sq, D = A_x.shape
    _, H, Sk, Dh = A_k_cache.shape
    F = B_w_gate.shape[1]
    P = 2 * Dh
    assert Sq == 1 and B == 4 and H % 2 == 0 and Sk % _GW == 0 and P % _CR == 0
    dt = A_k_cache.dtype
    f32 = jnp.float32

    kt = jnp.swapaxes(A_k_cache, 2, 3).reshape(B * H // 2, P, Sk)
    vt = jnp.swapaxes(A_v_cache, 2, 3).reshape(B * H // 2, P, Sk)

    out = pl.pallas_call(
        functools.partial(_body, B=B, H=H, Dh=Dh, Sk=Sk, D=D, F=F),
        in_specs=[pl.BlockSpec(memory_space=pl.ANY)] * 9,
        out_specs=pl.BlockSpec(memory_space=pltpu.VMEM),
        out_shape=jax.ShapeDtypeStruct((B, D), A_x.dtype),
        scratch_shapes=[
            pltpu.VMEM((_NB, P, _GW), dt),
            pltpu.VMEM((_NB, P, _GW), dt),
            pltpu.VMEM((D, P), dt),
            pltpu.VMEM((P, D), dt),
            pltpu.VMEM((D, F), dt),
            pltpu.VMEM((D, F), dt),
            pltpu.VMEM((F, D), dt),
            pltpu.VMEM((B, D), dt),
            pltpu.VMEM((D,), dt),
            pltpu.VMEM((2 * B, P), f32),
            pltpu.VMEM((2 * B, P), f32),
            pltpu.VMEM((2 * B, P), f32),
            pltpu.VMEM((2 * B, 1), f32),
            pltpu.VMEM((2 * B, 1), f32),
            pltpu.VMEM((2 * B, D), f32),
            pltpu.SemaphoreType.DMA((_NB,)),
            pltpu.SemaphoreType.DMA((_NB,)),
            pltpu.SemaphoreType.DMA((1,)),
            pltpu.SemaphoreType.DMA((1,)),
            pltpu.SemaphoreType.DMA((5,)),
        ],
        compiler_params=pltpu.CompilerParams(vmem_limit_bytes=48 * 1024 * 1024),
    )(A_x.reshape(B, D), kt, vt, A_wq, A_wo, B_w_r, B_w_gate, B_w_up, B_w_down)
    return out.reshape(B, Sq, D)
```

```python
import functools

import jax
import jax.numpy as jnp
import jax.experimental.pallas as pl
import jax.experimental.pallas.tpu as pltpu

_EPS = 1e-5
_NB = 3
_GW = 2048
_CW = 256
_CR = 80


def _layernorm(x):
    m = jnp.mean(x, axis=-1, keepdims=True)
    d = x - m
    v = jnp.mean(d * d, axis=-1, keepdims=True)
    return d / jnp.sqrt(v + _EPS)


def _dot(a, b):
    return jnp.dot(a, b, preferred_element_type=jnp.float32)


def _dot_nt(a, b):
    return jax.lax.dot_general(
        a, b, (((1,), (1,)), ((), ())), preferred_element_type=jnp.float32
    )


def _wait_all(buf, sem):
    pltpu.make_async_copy(buf, buf, sem).wait()


def _body(
    x_hbm, kt_hbm, vt_hbm, wq_hbm, wo_hbm, wr_hbm, wg_hbm, wu_hbm, wd_hbm,
    out_ref,
    kbuf, vbuf, wqbuf, wobuf, wgbuf, wubuf, wdbuf, xbuf, wrbuf,
    q_scr, o_scr, acc_scr, m_scr, l_scr, attn_scr,
    ksem, vsem, wqsem, wosem, msem,
    *, B, H, Dh, Sk, D, F,
):
    P = 2 * Dh
    n_pairs = H // 2
    G = Sk // _GW
    per_pair = B * G
    n_steps = n_pairs * per_pair
    scale = Dh ** -0.5

    def issue_kv(t):
        j = t % per_pair
        n = (j // G) * n_pairs + t // per_pair
        c0 = (j % G) * _GW
        slot = t % _NB

        half = _GW // _CW // 2

        def strip(i, carry):
            c = (i % half) * 2 + i // half
            dst = pl.ds(pl.multiple_of(c * _CW, _CW), _CW)
            src = pl.ds(pl.multiple_of(c0 + c * _CW, _CW), _CW)
            for r in range(0, P, _CR):
                rows = pl.ds(r, min(_CR, P - r))
                pltpu.make_async_copy(
                    kt_hbm.at[n, rows, src], kbuf.at[slot, rows, dst], ksem.at[slot]
                ).start(priority=0)
                pltpu.make_async_copy(
                    vt_hbm.at[n, rows, src], vbuf.at[slot, rows, dst], vsem.at[slot]
                ).start(priority=1)
            return carry

        jax.lax.fori_loop(0, _GW // _CW, strip, None)

    def issue_wq(p):
        cols = pl.ds(pl.multiple_of(p * P, P), P)
        for i, r in enumerate(range(0, D, 64)):
            pltpu.make_async_copy(
                wq_hbm.at[pl.ds(r, 64), cols], wqbuf.at[pl.ds(r, 64), :], wqsem.at[0]
            ).start(priority=i % 2)

    def issue_wo(p):
        for i, r in enumerate(range(0, P, 32)):
            pltpu.make_async_copy(
                wo_hbm.at[pl.ds(pl.multiple_of(p * P + r, 32), 32), :],
                wobuf.at[pl.ds(r, 32), :],
                wosem.at[0],
            ).start(priority=i % 2)

    def issue_gate_up():
        def piece(c, carry):
            rows = pl.ds(pl.multiple_of(c * 32, 32), 32)
            pltpu.make_async_copy(wg_hbm.at[rows, :], wgbuf.at[rows, :], msem.at[2]).start(priority=0)
            pltpu.make_async_copy(wu_hbm.at[rows, :], wubuf.at[rows, :], msem.at[3]).start(priority=1)
            return carry

        jax.lax.fori_loop(0, D // 32, piece, None)

    def issue_down():
        def piece(c, carry):
            for pr in range(2):
                rows = pl.ds(pl.multiple_of(c * 128 + pr * 64, 64), 64)
                pltpu.make_async_copy(wd_hbm.at[rows, :], wdbuf.at[rows, :], msem.at[4]).start(priority=pr)
            return carry

        jax.lax.fori_loop(0, F // 128, piece, None)

    x_cp = pltpu.make_async_copy(x_hbm, xbuf, msem.at[0])
    wr_cp = pltpu.make_async_copy(wr_hbm, wrbuf, msem.at[1])
    x_cp.start()
    wr_cp.start(priority=1)
    issue_wq(0)
    issue_kv(0)

    x_cp.wait()
    x4 = xbuf[...].astype(jnp.float32)
    x = jnp.concatenate([x4, x4], axis=0)
    xn = _layernorm(x).astype(jnp.bfloat16)
    row = jax.lax.broadcasted_iota(jnp.int32, (2 * B, P), 0)
    col = jax.lax.broadcasted_iota(jnp.int32, (2 * B, P), 1)
    diag = (row < B) == (col < Dh)
    attn_scr[...] = jnp.zeros_like(attn_scr)
    o_scr[...] = jnp.zeros_like(o_scr)

    for t in range(1, _NB):
        issue_kv(t)

    def step(t, carry):
        p = t // per_pair
        j = t % per_pair
        b = j // G
        g = j % G
        slot = t % _NB

        @pl.when(j == 0)
        def _():
            issue_wo(p)
            _wait_all(wqbuf, wqsem.at[0])
            q_scr[...] = jnp.where(diag, _dot(xn, wqbuf[...]), 0.0)

            @pl.when(p + 1 < n_pairs)
            def _():
                issue_wq(p + 1)

        @pl.when(g == 0)
        def _():
            m_scr[...] = jnp.full_like(m_scr, -jnp.inf)
            l_scr[...] = jnp.zeros_like(l_scr)
            acc_scr[...] = jnp.zeros_like(acc_scr)

        _wait_all(kbuf.at[slot], ksem.at[slot])
        _wait_all(vbuf.at[slot], vsem.at[slot])
        s = _dot(q_scr[...].astype(jnp.bfloat16), kbuf[slot]) * scale
        m_old = m_scr[...]
        m_new = jnp.maximum(m_old, jnp.max(s, axis=-1, keepdims=True))
        m_sub = jnp.where(m_new == -jnp.inf, 0.0, m_new)
        e = jnp.exp(s - m_sub)
        alpha = jnp.exp(m_old - m_sub)
        m_scr[...] = m_new
        l_scr[...] = alpha * l_scr[...] + jnp.sum(e, axis=-1, keepdims=True)
        acc_scr[...] = alpha * acc_scr[...] + _dot_nt(e.astype(jnp.bfloat16), vbuf[slot])

        @pl.when(t + _NB < n_steps)
        def _():
            issue_kv(t + _NB)

        @pl.when(t + _NB == n_steps)
        def _():
            issue_gate_up()

        @pl.when(t + 1 == n_steps)
        def _():
            issue_down()

        @pl.when(g == G - 1)
        def _():
            o = jnp.where(diag, acc_scr[...] / l_scr[...], 0.0)
            o_scr[...] = jnp.where(row % B == b, o, o_scr[...])

        @pl.when(j == per_pair - 1)
        def _():
            _wait_all(wobuf, wosem.at[0])
            attn_scr[...] += _dot(o_scr[...].astype(jnp.bfloat16), wobuf[...])

        return carry

    jax.lax.fori_loop(0, n_steps, step, None)

    attn = attn_scr[...]
    h = x + attn + pltpu.roll(attn, B, 0)
    hn = _layernorm(h)
    hb = hn.astype(jnp.bfloat16)
    wr_cp.wait()
    r = jnp.sum(hn * wrbuf[...].astype(jnp.float32).reshape(1, D), axis=-1, keepdims=True)
    _wait_all(wgbuf, msem.at[2])
    _wait_all(wubuf, msem.at[3])
    gate = _dot(hb, wgbuf[...])
    up = _dot(hb, wubuf[...])
    act = (gate * jax.nn.sigmoid(gate) * up).astype(jnp.bfloat16)
    _wait_all(wdbuf, msem.at[4])
    y = _dot(act, wdbuf[...]) * jax.nn.sigmoid(r)
    out = h + (hn + (hn * 0.0 + y))
    out_ref[...] = out[:B].astype(out_ref.dtype)


@jax.jit
def pallas_sequential_preLN__mha_block_cached__moe_arch_mod__decode_kernel(
    A_x: jax.Array,
    A_k_cache: jax.Array,
    A_v_cache: jax.Array,
    A_wq: jax.Array,
    A_wo: jax.Array,
    B_x: jax.Array,
    B_w_r: jax.Array,
    B_w_gate: jax.Array,
    B_w_up: jax.Array,
    B_w_down: jax.Array,
):
    del B_x
    B, Sq, D = A_x.shape
    _, H, Sk, Dh = A_k_cache.shape
    F = B_w_gate.shape[1]
    P = 2 * Dh
    assert Sq == 1 and B == 4 and H % 2 == 0 and Sk % _GW == 0 and P % 128 == 0
    dt = A_k_cache.dtype
    f32 = jnp.float32

    kt = jnp.swapaxes(A_k_cache, 2, 3).reshape(B * H // 2, P, Sk)
    vt = jnp.swapaxes(A_v_cache, 2, 3).reshape(B * H // 2, P, Sk)

    out = pl.pallas_call(
        functools.partial(_body, B=B, H=H, Dh=Dh, Sk=Sk, D=D, F=F),
        in_specs=[pl.BlockSpec(memory_space=pl.ANY)] * 9,
        out_specs=pl.BlockSpec(memory_space=pltpu.VMEM),
        out_shape=jax.ShapeDtypeStruct((B, D), A_x.dtype),
        scratch_shapes=[
            pltpu.VMEM((_NB, P, _GW), dt),
            pltpu.VMEM((_NB, P, _GW), dt),
            pltpu.VMEM((D, P), dt),
            pltpu.VMEM((P, D), dt),
            pltpu.VMEM((D, F), dt),
            pltpu.VMEM((D, F), dt),
            pltpu.VMEM((F, D), dt),
            pltpu.VMEM((B, D), dt),
            pltpu.VMEM((D,), dt),
            pltpu.VMEM((2 * B, P), f32),
            pltpu.VMEM((2 * B, P), f32),
            pltpu.VMEM((2 * B, P), f32),
            pltpu.VMEM((2 * B, 1), f32),
            pltpu.VMEM((2 * B, 1), f32),
            pltpu.VMEM((2 * B, D), f32),
            pltpu.SemaphoreType.DMA((_NB,)),
            pltpu.SemaphoreType.DMA((_NB,)),
            pltpu.SemaphoreType.DMA((1,)),
            pltpu.SemaphoreType.DMA((1,)),
            pltpu.SemaphoreType.DMA((5,)),
        ],
        compiler_params=pltpu.CompilerParams(vmem_limit_bytes=48 * 1024 * 1024),
    )(A_x.reshape(B, D), kt, vt, A_wq, A_wo, B_w_r, B_w_gate, B_w_up, B_w_down)
    return out.reshape(B, Sq, D)
```

```python
import functools

import jax
import jax.numpy as jnp
import jax.experimental.pallas as pl
import jax.experimental.pallas.tpu as pltpu

_EPS = 1e-5
_NB = 3
_GW = 2048
_CW = 256
_CR = 80
_FW = 256


def _layernorm(x):
    m = jnp.mean(x, axis=-1, keepdims=True)
    d = x - m
    v = jnp.mean(d * d, axis=-1, keepdims=True)
    return d / jnp.sqrt(v + _EPS)


def _dot(a, b):
    return jnp.dot(a, b, preferred_element_type=jnp.float32)


def _dot_nt(a, b):
    return jax.lax.dot_general(
        a, b, (((1,), (1,)), ((), ())), preferred_element_type=jnp.float32
    )


def _wait_all(buf, sem):
    pltpu.make_async_copy(buf, buf, sem).wait()


def _body(
    x_hbm, kt_hbm, vt_hbm, wq_hbm, wo_hbm, wr_hbm, wg_hbm, wu_hbm, wd_hbm,
    out_ref,
    kbuf, vbuf, wqbuf, wobuf, wgbuf, wubuf, wdbuf, xbuf, wrbuf,
    q_scr, o_scr, acc_scr, m_scr, l_scr, attn_scr,
    ksem, vsem, wqsem, wosem, msem, gsem, usem, dsem,
    *, B, H, Dh, Sk, D, F,
):
    P = 2 * Dh
    n_pairs = H // 2
    G = Sk // _GW
    per_pair = B * G
    n_steps = n_pairs * per_pair
    NF = F // _FW
    scale = Dh ** -0.5

    def issue_kv(t):
        j = t % per_pair
        n = (j // G) * n_pairs + t // per_pair
        c0 = (j % G) * _GW
        slot = t % _NB

        half = _GW // _CW // 2

        def cols(i):
            c = ((i % half) * 2 + (i // half) % 2) * _CW
            return (
                pl.ds(pl.multiple_of(c0 + c, _CW), _CW),
                pl.ds(pl.multiple_of(c, _CW), _CW),
            )

        def strip(i, carry):
            k_src, k_dst = cols(i)
            v_src, v_dst = cols(i + 2)
            for r in range(0, P, _CR):
                rows = pl.ds(r, min(_CR, P - r))
                pltpu.make_async_copy(
                    kt_hbm.at[n, rows, k_src], kbuf.at[slot, rows, k_dst], ksem.at[slot]
                ).start(priority=0)
                pltpu.make_async_copy(
                    vt_hbm.at[n, rows, v_src], vbuf.at[slot, rows, v_dst], vsem.at[slot]
                ).start(priority=1)
            return carry

        jax.lax.fori_loop(0, _GW // _CW, strip, None)

    def issue_wq(p):
        cols = pl.ds(pl.multiple_of(p * P, P), P)
        for i, r in enumerate(range(0, D, 64)):
            pltpu.make_async_copy(
                wq_hbm.at[pl.ds(r, 64), cols], wqbuf.at[pl.ds(r, 64), :], wqsem.at[0]
            ).start(priority=i % 2)

    def issue_wo(p):
        for i, r in enumerate(range(0, P, 64)):
            pltpu.make_async_copy(
                wo_hbm.at[pl.ds(pl.multiple_of(p * P + r, 64), 64), :],
                wobuf.at[pl.ds(r, 64), :],
                wosem.at[0],
            ).start(priority=i % 2)

    def issue_gate_up(lo, hi):
        def piece(f, carry):
            cols = pl.ds(pl.multiple_of(f * _FW, _FW), _FW)
            for r in range(0, D, _CR):
                rows = pl.ds(r, _CR)
                pltpu.make_async_copy(
                    wg_hbm.at[rows, cols], wgbuf.at[f, rows, :], gsem.at[f]
                ).start(priority=0)
                pltpu.make_async_copy(
                    wu_hbm.at[rows, cols], wubuf.at[f, rows, :], usem.at[f]
                ).start(priority=1)
            return carry

        jax.lax.fori_loop(lo, hi, piece, None)

    def issue_down():
        def piece(f, carry):
            for i, r in enumerate(range(0, _FW, 32)):
                pltpu.make_async_copy(
                    wd_hbm.at[pl.ds(pl.multiple_of(f * _FW + r, 32), 32), :],
                    wdbuf.at[f, pl.ds(r, 32), :],
                    dsem.at[f],
                ).start(priority=i % 2)
            return carry

        jax.lax.fori_loop(0, NF, piece, None)

    x_cp = pltpu.make_async_copy(x_hbm, xbuf, msem.at[0])
    wr_cp = pltpu.make_async_copy(wr_hbm, wrbuf, msem.at[1])
    x_cp.start()
    wr_cp.start(priority=1)
    issue_wq(0)
    issue_kv(0)

    x_cp.wait()
    x4 = xbuf[...].astype(jnp.float32)
    x = jnp.concatenate([x4, x4], axis=0)
    xn = _layernorm(x).astype(jnp.bfloat16)
    row = jax.lax.broadcasted_iota(jnp.int32, (2 * B, P), 0)
    col = jax.lax.broadcasted_iota(jnp.int32, (2 * B, P), 1)
    diag = (row < B) == (col < Dh)
    attn_scr[...] = jnp.zeros_like(attn_scr)
    o_scr[...] = jnp.zeros_like(o_scr)

    for t in range(1, _NB):
        issue_kv(t)

    def step(t, carry):
        p = t // per_pair
        j = t % per_pair
        b = j // G
        g = j % G
        slot = t % _NB

        @pl.when(j == 0)
        def _():
            issue_wo(p)
            _wait_all(wqbuf, wqsem.at[0])
            q_scr[...] = jnp.where(diag, _dot(xn, wqbuf[...]), 0.0)

            @pl.when(p + 1 < n_pairs)
            def _():
                issue_wq(p + 1)

        @pl.when(g == 0)
        def _():
            m_scr[...] = jnp.full_like(m_scr, -jnp.inf)
            l_scr[...] = jnp.zeros_like(l_scr)
            acc_scr[...] = jnp.zeros_like(acc_scr)

        _wait_all(kbuf.at[slot], ksem.at[slot])
        _wait_all(vbuf.at[slot], vsem.at[slot])
        s = _dot(q_scr[...].astype(jnp.bfloat16), kbuf[slot]) * scale
        m_old = m_scr[...]
        m_new = jnp.maximum(m_old, jnp.max(s, axis=-1, keepdims=True))
        m_sub = jnp.where(m_new == -jnp.inf, 0.0, m_new)
        e = jnp.exp(s - m_sub)
        alpha = jnp.exp(m_old - m_sub)
        m_scr[...] = m_new
        l_scr[...] = alpha * l_scr[...] + jnp.sum(e, axis=-1, keepdims=True)
        acc_scr[...] = alpha * acc_scr[...] + _dot_nt(e.astype(jnp.bfloat16), vbuf[slot])

        @pl.when(t + _NB < n_steps)
        def _():
            issue_kv(t + _NB)

        @pl.when(t + 3 == n_steps)
        def _():
            issue_gate_up(0, NF // 2)

        @pl.when(t + 2 == n_steps)
        def _():
            issue_gate_up(NF // 2, NF)

        @pl.when(t + 1 == n_steps)
        def _():
            issue_down()

        @pl.when(g == G - 1)
        def _():
            o = jnp.where(diag, acc_scr[...] / l_scr[...], 0.0)
            o_scr[...] = jnp.where(row % B == b, o, o_scr[...])

        @pl.when(j == per_pair - 1)
        def _():
            _wait_all(wobuf, wosem.at[0])
            attn_scr[...] += _dot(o_scr[...].astype(jnp.bfloat16), wobuf[...])

        return carry

    jax.lax.fori_loop(0, n_steps, step, None)

    attn = attn_scr[...]
    h = x + attn + pltpu.roll(attn, B, 0)
    hn = _layernorm(h)
    hb = hn.astype(jnp.bfloat16)
    wr_cp.wait()
    r = jnp.sum(hn * wrbuf[...].astype(jnp.float32).reshape(1, D), axis=-1, keepdims=True)
    acts = []
    for f in range(NF):
        _wait_all(wgbuf.at[f], gsem.at[f])
        _wait_all(wubuf.at[f], usem.at[f])
        gate = _dot(hb, wgbuf[f])
        up = _dot(hb, wubuf[f])
        acts.append((gate * jax.nn.sigmoid(gate) * up).astype(jnp.bfloat16))
    y = jnp.zeros((2 * B, D), jnp.float32)
    for f in range(NF):
        _wait_all(wdbuf.at[f], dsem.at[f])
        y = y + _dot(acts[f], wdbuf[f])
    y = y * jax.nn.sigmoid(r)
    out = h + (hn + (hn * 0.0 + y))
    out_ref[...] = out[:B].astype(out_ref.dtype)


@jax.jit
def pallas_sequential_preLN__mha_block_cached__moe_arch_mod__decode_kernel(
    A_x: jax.Array,
    A_k_cache: jax.Array,
    A_v_cache: jax.Array,
    A_wq: jax.Array,
    A_wo: jax.Array,
    B_x: jax.Array,
    B_w_r: jax.Array,
    B_w_gate: jax.Array,
    B_w_up: jax.Array,
    B_w_down: jax.Array,
):
    del B_x
    B, Sq, D = A_x.shape
    _, H, Sk, Dh = A_k_cache.shape
    F = B_w_gate.shape[1]
    P = 2 * Dh
    assert Sq == 1 and B == 4 and H % 2 == 0 and Sk % _GW == 0 and P % 128 == 0
    assert F % _FW == 0 and D % _CR == 0 and D % 64 == 0
    dt = A_k_cache.dtype
    f32 = jnp.float32

    kt = jnp.swapaxes(A_k_cache, 2, 3).reshape(B * H // 2, P, Sk)
    vt = jnp.swapaxes(A_v_cache, 2, 3).reshape(B * H // 2, P, Sk)

    out = pl.pallas_call(
        functools.partial(_body, B=B, H=H, Dh=Dh, Sk=Sk, D=D, F=F),
        in_specs=[pl.BlockSpec(memory_space=pl.ANY)] * 9,
        out_specs=pl.BlockSpec(memory_space=pltpu.VMEM),
        out_shape=jax.ShapeDtypeStruct((B, D), A_x.dtype),
        scratch_shapes=[
            pltpu.VMEM((_NB, P, _GW), dt),
            pltpu.VMEM((_NB, P, _GW), dt),
            pltpu.VMEM((D, P), dt),
            pltpu.VMEM((P, D), dt),
            pltpu.VMEM((F // _FW, D, _FW), dt),
            pltpu.VMEM((F // _FW, D, _FW), dt),
            pltpu.VMEM((F // _FW, _FW, D), dt),
            pltpu.VMEM((B, D), dt),
            pltpu.VMEM((D,), dt),
            pltpu.VMEM((2 * B, P), f32),
            pltpu.VMEM((2 * B, P), f32),
            pltpu.VMEM((2 * B, P), f32),
            pltpu.VMEM((2 * B, 1), f32),
            pltpu.VMEM((2 * B, 1), f32),
            pltpu.VMEM((2 * B, D), f32),
            pltpu.SemaphoreType.DMA((_NB,)),
            pltpu.SemaphoreType.DMA((_NB,)),
            pltpu.SemaphoreType.DMA((1,)),
            pltpu.SemaphoreType.DMA((1,)),
            pltpu.SemaphoreType.DMA((2,)),
            pltpu.SemaphoreType.DMA((F // _FW,)),
            pltpu.SemaphoreType.DMA((F // _FW,)),
            pltpu.SemaphoreType.DMA((F // _FW,)),
        ],
        compiler_params=pltpu.CompilerParams(vmem_limit_bytes=48 * 1024 * 1024),
    )(A_x.reshape(B, D), kt, vt, A_wq, A_wo, B_w_r, B_w_gate, B_w_up, B_w_down)
    return out.reshape(B, Sq, D)
```

```python
import functools

import jax
import jax.numpy as jnp
import jax.experimental.pallas as pl
import jax.experimental.pallas.tpu as pltpu

_EPS = 1e-5
_NB = 3
_GW = 2048
_CW = 256
_RB = 48
_CR = 80
_FW = 256


def _layernorm(x):
    m = jnp.mean(x, axis=-1, keepdims=True)
    d = x - m
    v = jnp.mean(d * d, axis=-1, keepdims=True)
    return d / jnp.sqrt(v + _EPS)


def _dot(a, b):
    return jnp.dot(a, b, preferred_element_type=jnp.float32)


def _dot_nt(a, b):
    return jax.lax.dot_general(
        a, b, (((1,), (1,)), ((), ())), preferred_element_type=jnp.float32
    )


def _wait_all(buf, sem):
    pltpu.make_async_copy(buf, buf, sem).wait()


def _body(
    x_hbm, kt_hbm, vt_hbm, wq_hbm, wo_hbm, wr_hbm, wg_hbm, wu_hbm, wd_hbm,
    out_ref,
    kbuf, vbuf, wqbuf, wobuf, wgbuf, wubuf, wdbuf, xbuf, wrbuf,
    q_scr, o_scr, acc_scr, m_scr, l_scr, attn_scr,
    ksem, vsem, wqsem, wosem, msem, gsem, usem, dsem,
    *, B, H, Dh, Sk, D, F,
):
    P = 2 * Dh
    n_pairs = H // 2
    G = Sk // _GW
    per_pair = B * G
    n_steps = n_pairs * per_pair
    NF = F // _FW
    scale = Dh ** -0.5

    def issue_kv(t):
        j = t % per_pair
        n = (j // G) * n_pairs + t // per_pair
        c0 = (j % G) * _GW
        slot = t % _NB

        def cols(i, second):
            c = ((i % 2) * 4 + (i // 2) % 2 + 2 * second) * _CW
            return (
                pl.ds(pl.multiple_of(c0 + c, _CW), _CW),
                pl.ds(pl.multiple_of(c, _CW), _CW),
            )

        def strip_pair(i, carry):
            for r in range(0, _RB, 8):
                rows = pl.ds(r, 8)
                for second in range(2):
                    k_src, k_dst = cols(i, second)
                    v_src, v_dst = cols(i + 2, second)
                    pltpu.make_async_copy(
                        kt_hbm.at[n, :, rows, k_src], kbuf.at[slot, :, rows, k_dst], ksem.at[slot]
                    ).start(priority=0)
                    pltpu.make_async_copy(
                        vt_hbm.at[n, :, rows, v_src], vbuf.at[slot, :, rows, v_dst], vsem.at[slot]
                    ).start(priority=1)
            return carry

        jax.lax.fori_loop(0, 4, strip_pair, None)

    def issue_wq(p):
        cols = pl.ds(pl.multiple_of(p * P, P), P)
        for i, r in enumerate(range(0, D, 64)):
            pltpu.make_async_copy(
                wq_hbm.at[pl.ds(r, 64), cols], wqbuf.at[pl.ds(r, 64), :], wqsem.at[0]
            ).start(priority=i % 2)

    def issue_wo(p):
        for i, r in enumerate(range(0, P, 64)):
            pltpu.make_async_copy(
                wo_hbm.at[pl.ds(pl.multiple_of(p * P + r, 64), 64), :],
                wobuf.at[pl.ds(r, 64), :],
                wosem.at[0],
            ).start(priority=i % 2)

    def issue_gate_up(lo, hi):
        def piece(f, carry):
            cols = pl.ds(pl.multiple_of(f * _FW, _FW), _FW)
            for r in range(0, D, _CR):
                rows = pl.ds(r, _CR)
                pltpu.make_async_copy(
                    wg_hbm.at[rows, cols], wgbuf.at[f, rows, :], gsem.at[f]
                ).start(priority=0)
                pltpu.make_async_copy(
                    wu_hbm.at[rows, cols], wubuf.at[f, rows, :], usem.at[f]
                ).start(priority=1)
            return carry

        jax.lax.fori_loop(lo, hi, piece, None)

    def issue_down():
        def piece(f, carry):
            for i, r in enumerate(range(0, _FW, 32)):
                pltpu.make_async_copy(
                    wd_hbm.at[pl.ds(pl.multiple_of(f * _FW + r, 32), 32), :],
                    wdbuf.at[f, pl.ds(r, 32), :],
                    dsem.at[f],
                ).start(priority=i % 2)
            return carry

        jax.lax.fori_loop(0, NF, piece, None)

    x_cp = pltpu.make_async_copy(x_hbm, xbuf, msem.at[0])
    wr_cp = pltpu.make_async_copy(wr_hbm, wrbuf, msem.at[1])
    x_cp.start()
    wr_cp.start(priority=1)
    issue_wq(0)
    issue_kv(0)

    x_cp.wait()
    x4 = xbuf[...].astype(jnp.float32)
    x = jnp.concatenate([x4, x4], axis=0)
    xn = _layernorm(x).astype(jnp.bfloat16)
    row = jax.lax.broadcasted_iota(jnp.int32, (2 * B, P), 0)
    col = jax.lax.broadcasted_iota(jnp.int32, (2 * B, P), 1)
    diag = (row < B) == (col < Dh)
    attn_scr[...] = jnp.zeros_like(attn_scr)
    o_scr[...] = jnp.zeros_like(o_scr)

    jax.lax.fori_loop(1, _NB, lambda t, carry: issue_kv(t), None)

    def step(t, carry):
        p = t // per_pair
        j = t % per_pair
        b = j // G
        g = j % G
        slot = t % _NB

        @pl.when(j == 0)
        def _():
            issue_wo(p)
            _wait_all(wqbuf, wqsem.at[0])
            q_scr[...] = jnp.where(diag, _dot(xn, wqbuf[...]), 0.0)

            @pl.when(p + 1 < n_pairs)
            def _():
                issue_wq(p + 1)

        @pl.when(g == 0)
        def _():
            m_scr[...] = jnp.full_like(m_scr, -jnp.inf)
            l_scr[...] = jnp.zeros_like(l_scr)
            acc_scr[...] = jnp.zeros_like(acc_scr)

        _wait_all(kbuf.at[slot], ksem.at[slot])
        s = _dot(q_scr[...].astype(jnp.bfloat16), kbuf[slot].reshape(P, _GW)) * scale
        m_old = m_scr[...]
        m_new = jnp.maximum(m_old, jnp.max(s, axis=-1, keepdims=True))
        m_sub = jnp.where(m_new == -jnp.inf, 0.0, m_new)
        e = jnp.exp(s - m_sub)
        alpha = jnp.exp(m_old - m_sub)
        m_scr[...] = m_new
        l_scr[...] = alpha * l_scr[...] + jnp.sum(e, axis=-1, keepdims=True)
        _wait_all(vbuf.at[slot], vsem.at[slot])
        pv = _dot_nt(e.astype(jnp.bfloat16), vbuf[slot].reshape(P, _GW))
        acc_scr[...] = alpha * acc_scr[...] + pv

        @pl.when(t + _NB < n_steps)
        def _():
            issue_kv(t + _NB)

        @pl.when(t + 3 == n_steps)
        def _():
            issue_gate_up(0, NF // 2)

        @pl.when(t + 2 == n_steps)
        def _():
            issue_gate_up(NF // 2, NF)

        @pl.when(t + 1 == n_steps)
        def _():
            issue_down()

        @pl.when(g == G - 1)
        def _():
            o = jnp.where(diag, acc_scr[...] / l_scr[...], 0.0)
            o_scr[...] = jnp.where(row % B == b, o, o_scr[...])

        @pl.when(j == per_pair - 1)
        def _():
            _wait_all(wobuf, wosem.at[0])
            attn_scr[...] += _dot(o_scr[...].astype(jnp.bfloat16), wobuf[...])

        return carry

    jax.lax.fori_loop(0, n_steps, step, None)

    attn = attn_scr[...]
    h = x + attn + pltpu.roll(attn, B, 0)
    hn = _layernorm(h)
    hb = hn.astype(jnp.bfloat16)
    wr_cp.wait()
    r = jnp.sum(hn * wrbuf[...].astype(jnp.float32).reshape(1, D), axis=-1, keepdims=True)
    acts = []
    for f in range(NF):
        _wait_all(wgbuf.at[f], gsem.at[f])
        _wait_all(wubuf.at[f], usem.at[f])
        gate = _dot(hb, wgbuf[f])
        up = _dot(hb, wubuf[f])
        acts.append((gate * jax.nn.sigmoid(gate) * up).astype(jnp.bfloat16))
    y = jnp.zeros((2 * B, D), jnp.float32)
    for f in range(NF):
        _wait_all(wdbuf.at[f], dsem.at[f])
        y = y + _dot(acts[f], wdbuf[f])
    y = y * jax.nn.sigmoid(r)
    out = h + (hn + (hn * 0.0 + y))
    out_ref[...] = out[:B].astype(out_ref.dtype)


@jax.jit
def pallas_sequential_preLN__mha_block_cached__moe_arch_mod__decode_kernel(
    A_x: jax.Array,
    A_k_cache: jax.Array,
    A_v_cache: jax.Array,
    A_wq: jax.Array,
    A_wo: jax.Array,
    B_x: jax.Array,
    B_w_r: jax.Array,
    B_w_gate: jax.Array,
    B_w_up: jax.Array,
    B_w_down: jax.Array,
):
    del B_x
    B, Sq, D = A_x.shape
    _, H, Sk, Dh = A_k_cache.shape
    F = B_w_gate.shape[1]
    P = 2 * Dh
    assert Sq == 1 and B == 4 and H % 2 == 0 and Sk % _GW == 0 and P % 128 == 0
    assert P % _RB == 0 and _GW == 8 * _CW and F % _FW == 0 and D % _CR == 0 and D % 64 == 0
    dt = A_k_cache.dtype
    f32 = jnp.float32

    kt = jnp.swapaxes(A_k_cache, 2, 3).reshape(B * H // 2, P // _RB, _RB, Sk)
    vt = jnp.swapaxes(A_v_cache, 2, 3).reshape(B * H // 2, P // _RB, _RB, Sk)

    out = pl.pallas_call(
        functools.partial(_body, B=B, H=H, Dh=Dh, Sk=Sk, D=D, F=F),
        in_specs=[pl.BlockSpec(memory_space=pl.ANY)] * 9,
        out_specs=pl.BlockSpec(memory_space=pltpu.VMEM),
        out_shape=jax.ShapeDtypeStruct((B, D), A_x.dtype),
        scratch_shapes=[
            pltpu.VMEM((_NB, P // _RB, _RB, _GW), dt),
            pltpu.VMEM((_NB, P // _RB, _RB, _GW), dt),
            pltpu.VMEM((D, P), dt),
            pltpu.VMEM((P, D), dt),
            pltpu.VMEM((F // _FW, D, _FW), dt),
            pltpu.VMEM((F // _FW, D, _FW), dt),
            pltpu.VMEM((F // _FW, _FW, D), dt),
            pltpu.VMEM((B, D), dt),
            pltpu.VMEM((D,), dt),
            pltpu.VMEM((2 * B, P), f32),
            pltpu.VMEM((2 * B, P), f32),
            pltpu.VMEM((2 * B, P), f32),
            pltpu.VMEM((2 * B, 1), f32),
            pltpu.VMEM((2 * B, 1), f32),
            pltpu.VMEM((2 * B, D), f32),
            pltpu.SemaphoreType.DMA((_NB,)),
            pltpu.SemaphoreType.DMA((_NB,)),
            pltpu.SemaphoreType.DMA((1,)),
            pltpu.SemaphoreType.DMA((1,)),
            pltpu.SemaphoreType.DMA((2,)),
            pltpu.SemaphoreType.DMA((F // _FW,)),
            pltpu.SemaphoreType.DMA((F // _FW,)),
            pltpu.SemaphoreType.DMA((F // _FW,)),
        ],
        compiler_params=pltpu.CompilerParams(vmem_limit_bytes=48 * 1024 * 1024),
    )(A_x.reshape(B, D), kt, vt, A_wq, A_wo, B_w_r, B_w_gate, B_w_up, B_w_down)
    return out.reshape(B, Sq, D)
```
